```python
import os as _os
_os.environ.setdefault("JAX_PLATFORMS", "cpu")
import jax
import jax.numpy as jnp

def _softmax(x, axis=-1):
    return jax.nn.softmax(x, axis=axis)
def _gelu(x):
    return jax.nn.gelu(x, approximate=True)
def _silu(x):
    return jax.nn.silu(x)
def _sigmoid(x):
    return jax.nn.sigmoid(x)
def _layernorm(x, axis=-1, eps=1e-5):
    m = jnp.mean(x, axis=axis, keepdims=True)
    v = jnp.var(x, axis=axis, keepdims=True)
    return (x - m) / jnp.sqrt(v + eps)
def _scatter_add(tgt, idx, src, axis=0):
    return tgt.at[idx].add(src)
def _segment_sum(src, seg, n):
    return jax.ops.segment_sum(src, seg, n)
class _Rng:
    def __init__(self, key):
        self._k = key
    def _next(self):
        self._k, sub = jax.random.split(self._k)
        return sub
    def normal(self, shape):
        return jax.random.normal(self._next(), shape, dtype=jnp.bfloat16)
    def randint(self, lo, hi, shape):
        return jax.random.randint(self._next(), shape, lo, hi, dtype=jnp.int32)
    def uniform(self, shape, lo=0.0, hi=1.0):
        return jax.random.uniform(self._next(), shape, jnp.bfloat16, lo, hi)
    def permutation(self, n):
        return jax.random.permutation(self._next(), n)


kernel_name = 'concat_heads__mha_block__linear_attn_block__prompt'

def setup_inputs():
    _rng = _Rng(jax.random.key(int.from_bytes(__import__("os").urandom(4), "little")))
    _w = (lambda a: (lambda t: t.astype(jnp.bfloat16) if jnp.issubdtype(t.dtype, jnp.floating) else t)(jnp.asarray(a)))
    def _A_setup():
        B, S, D, H = 1, 2048, 1024, 32
        return {
            "x": _w((lambda *s: _rng.normal(s) * 0.2)(B, S, D)),
            "wqkv": _w((lambda *s: _rng.normal(s) * 0.2)(D, 3 * D)),
            "wo": _w((lambda *s: _rng.normal(s) * 0.05)(D, D)),
        }
    _A_in = _A_setup()

    def _B_setup():
        B, S, D = 1, 2048, 1024
        return {
            "x": _w((lambda *s: _rng.normal(s) * 0.05)(B, S, D)),
            "wqkv": _w((lambda *s: _rng.normal(s) * 1.6)(D, 3 * D)),
            "wo": _w((lambda *s: _rng.normal(s) * 0.1)(D, D)),
        }
    _B_in = _B_setup()

    return {
        "A_x": _A_in["x"],
        "A_wqkv": _A_in["wqkv"],
        "A_wo": _A_in["wo"],
        "B_x": _B_in["x"],
        "B_wqkv": _B_in["wqkv"],
        "B_wo": _B_in["wo"],
    }

def reference(A_x, A_wqkv, A_wo, B_x, B_wqkv, B_wo):
    def _A_ref(x, wqkv, wo):
        B, S, D = x.shape
        H = 32
        Dh = D // H
        qkv = (lambda x, *d: x.transpose(*d))((x @ wqkv).reshape(B, S, 3, H, Dh), 2, 0, 3, 1, 4)
        q, k, v = qkv[0], qkv[1], qkv[2]
        scores = jnp.einsum("bhqd,bhkd->bhqk", q, k) * (Dh ** -0.5)
        p = _softmax(scores, axis=-1)
        o = jnp.einsum("bhqk,bhkd->bhqd", p, v)
        return (lambda x, *d: x.transpose(*d))(o, 0, 2, 1, 3).reshape(B, S, D) @ wo

    def _B_ref(x, wqkv, wo):
        B, S, D = x.shape
        H = 32; Dh = D // H
        qkv = (lambda x, *d: x.transpose(*d))((x @ wqkv).reshape(B, S, 3, H, Dh), 2, 0, 3, 1, 4)
        q, k, v = qkv[0], qkv[1], qkv[2]
        phi = lambda t: jnp.where(t > 0, t + 1, jnp.exp(t)) + 1e-6
        pq, pk = phi(q), phi(k)
        kv = jnp.einsum("bhsd,bhse->bhde", pk, v)
        z = jnp.einsum("bhsd->bhd", pk)
        num = jnp.einsum("bhqd,bhde->bhqe", pq, kv)
        den = jnp.einsum("bhqd,bhd->bhq", pq, z)[..., None] + 1e-6
        o = num / den
        return (lambda x, *d: x.transpose(*d))(o, 0, 2, 1, 3).reshape(B, S, D) @ wo

    a = _A_ref(A_x, A_wqkv, A_wo)
    b = _B_ref(B_x, B_wqkv, B_wo)
    return jnp.concatenate([a, b], axis=-1)
```

```python
import math

import jax
import jax.numpy as jnp
from jax import lax
import jax.experimental.pallas as pl
import jax.experimental.pallas.tpu as pltpu

S = 2048
D = 1024
DH = 32
G = 8
TQ = 128
NQ = S // TQ
CK = 128
NC = S // CK
W = 4 * TQ
RB = 512
NRB = S // RB
CPB = RB // CK

F32 = jnp.float32
BF16 = jnp.bfloat16
NT = (((1,), (1,)), ((), ()))
QSCALE = (DH ** -0.5) * math.log2(math.e)


def _dot(a, b):
    return jnp.dot(a, b, preferred_element_type=F32)


def _dot_nt(a, b):
    return lax.dot_general(a, b, NT, preferred_element_type=F32)


def _phi(t):
    return jnp.where(t > 0, t + 1.0, jnp.exp(t)) + 1e-6


def _kernel(xa_hbm, wa_hbm, woa_hbm, xb_hbm, wb_hbm, wob_hbm, out_hbm,
            xa, wa, woa, xb, wb, wob,
            q_s, k_s, vt_s, o_s, sbufs, m_s, l_s,
            kvt_s, z_s, kvz_s, ostage, zero_ref, in_sems, out_sems):
    copies = [
        pltpu.make_async_copy(xa_hbm.at[0], xa, in_sems.at[0]),
        pltpu.make_async_copy(wa_hbm, wa, in_sems.at[1]),
        pltpu.make_async_copy(xb_hbm.at[0], xb, in_sems.at[2]),
        pltpu.make_async_copy(wb_hbm, wb, in_sems.at[3]),
        pltpu.make_async_copy(woa_hbm, woa, in_sems.at[4]),
        pltpu.make_async_copy(wob_hbm, wob, in_sems.at[5]),
    ]
    for cp in copies:
        cp.start()
    zero_ref[0] = 0
    copies[0].wait()
    copies[1].wait()

    def qkv_a(rb, carry):
        rows = pl.ds(pl.multiple_of(rb * RB, RB), RB)
        xblk = xa[rows, :]
        q_s[rows, :] = (_dot(xblk, wa[:, 0:D]) * QSCALE).astype(BF16)
        k_s[rows, :] = _dot(xblk, wa[:, D:2 * D]).astype(BF16)
        vt_s[rb] = _dot(xblk, wa[:, 2 * D:3 * D]).T.astype(BF16)
        return carry

    lax.fori_loop(0, NRB, qkv_a, 0)

    lane_head = lax.broadcasted_iota(jnp.int32, (TQ, 128), 1) // DH

    def get_qm(j, g):
        qf = q_s[pl.ds(pl.multiple_of(j * TQ, TQ), TQ), g * 128:(g + 1) * 128].astype(F32)
        return jnp.concatenate(
            [jnp.where(lane_head == h, qf, 0.0) for h in range(4)], axis=0).astype(BF16)

    def a_chunk(g, qm, c, macc):
        kc = k_s[c * CK:(c + 1) * CK, g * 128:(g + 1) * 128]
        s = _dot_nt(kc, qm)
        sbufs[g, c * CK:(c + 1) * CK, :] = s
        cm = jnp.max(s.reshape(CK // 8, 8, W), axis=0)
        return cm if macc is None else jnp.maximum(macc, cm)

    def a_final(g, macc):
        m_s[g] = jnp.max(macc, axis=0, keepdims=True)

    def b_chunk(g, c, m, accs):
        s = sbufs[g, c * CK:(c + 1) * CK, :]
        p = jnp.exp2(s - m)
        l_s[g, c] = jnp.sum(p.reshape(CK // 8, 8, W), axis=0)
        new = []
        for h in range(4):
            r0 = (g * 4 + h) * DH
            c0 = (c % CPB) * CK
            vt = vt_s[c // CPB, r0:r0 + DH, c0:c0 + CK]
            d = _dot(vt, p[:, h * TQ:(h + 1) * TQ].astype(BF16))
            new.append(d if accs is None else accs[h] + d)
        return new

    def b_final(j, g, accs, z):
        l = jnp.sum(jnp.sum(l_s[g, pl.ds(z, NC)], axis=0), axis=0, keepdims=True)
        r = 1.0 / l
        ot = jnp.concatenate(
            [accs[h] * r[:, h * TQ:(h + 1) * TQ] for h in range(4)], axis=0)
        o_s[pl.ds(pl.multiple_of(j * TQ, TQ), TQ), g * 128:(g + 1) * 128] = ot.T.astype(BF16)

    def a_only(j):
        for g in range(G):
            qm = get_qm(j, g)
            macc = None
            for c in range(NC):
                macc = a_chunk(g, qm, c, macc)
            a_final(g, macc)

    def att_step(j, do_a):
        z = zero_ref[0]
        for g in range(G):
            m = m_s[g]
            qm = get_qm(j + 1, g) if do_a else None
            accs = None
            macc = None
            for c in range(NC):
                accs = b_chunk(g, c, m, accs)
                if do_a:
                    macc = a_chunk(g, qm, c, macc)
            b_final(j, g, accs, z)
            if do_a:
                a_final(g, macc)

    a_only(0)

    def att_body(j, carry):
        att_step(j, True)
        return carry

    lax.fori_loop(0, NQ - 1, att_body, 0)
    att_step(NQ - 1, False)

    for cp in copies[2:]:
        cp.wait()

    kvt_s[...] = jnp.zeros(kvt_s.shape, F32)
    z_s[...] = jnp.zeros(z_s.shape, F32)

    def kv_b(rb, carry):
        rows = pl.ds(pl.multiple_of(rb * RB, RB), RB)
        xblk = xb[rows, :]
        k = _dot(xblk, wb[:, D:2 * D]).astype(BF16).astype(F32)
        pk = _phi(k).astype(BF16)
        z_s[...] += jnp.sum(pk.astype(F32).reshape(RB // 8, 8, D), axis=0)
        vt = _dot(xblk, wb[:, 2 * D:3 * D]).T.astype(BF16)
        for g in range(G):
            kvt_s[g] += _dot(vt[g * 128:(g + 1) * 128, :], pk[:, g * 128:(g + 1) * 128])
        return carry

    lax.fori_loop(0, NRB, kv_b, 0)

    bd = (lax.broadcasted_iota(jnp.int32, (128, 128), 0) // DH
          == lax.broadcasted_iota(jnp.int32, (128, 128), 1) // DH)
    zrow = jnp.sum(z_s[...], axis=0, keepdims=True)
    for g in range(G):
        kvz_s[g, 0:128, :] = jnp.where(bd, kvt_s[g], 0.0).astype(BF16)
        zg = jnp.broadcast_to(zrow[:, g * 128:(g + 1) * 128], (128, 128))
        kvz_s[g, 128:256, :] = jnp.where(bd, zg, 0.0).astype(BF16)

    def out_copy(rb):
        rows = pl.ds(pl.multiple_of(rb * RB, RB), RB)
        return pltpu.make_async_copy(ostage.at[rows, :], out_hbm.at[0, rows, :], out_sems.at[rb])

    def out_b(rb, carry):
        rows = pl.ds(pl.multiple_of(rb * RB, RB), RB)
        xblk = xb[rows, :]
        q = _dot(xblk, wb[:, 0:D]).astype(BF16).astype(F32)
        pq = _phi(q).astype(BF16)
        os_ = []
        for g in range(G):
            nd = _dot_nt(pq[:, g * 128:(g + 1) * 128], kvz_s[g])
            os_.append((nd[:, 0:128] / (nd[:, 128:256] + 1e-6)).astype(BF16))
        ob = jnp.concatenate(os_, axis=1)
        ostage[rows, D:2 * D] = _dot(ob, wob[...]).astype(BF16)
        ostage[rows, 0:D] = _dot(o_s[rows, :], woa[...]).astype(BF16)
        out_copy(rb).start()
        return carry

    lax.fori_loop(0, NRB, out_b, 0)
    for rb in range(NRB):
        out_copy(rb).wait()


@jax.jit
def pallas_concat_heads__mha_block__linear_attn_block__prompt_kernel(
    A_x: jax.Array,
    A_wqkv: jax.Array,
    A_wo: jax.Array,
    B_x: jax.Array,
    B_wqkv: jax.Array,
    B_wo: jax.Array,
):
    any_spec = pl.BlockSpec(memory_space=pl.ANY)
    scratch = [
        pltpu.VMEM((S, D), BF16),
        pltpu.VMEM((D, 3 * D), BF16),
        pltpu.VMEM((D, D), BF16),
        pltpu.VMEM((S, D), BF16),
        pltpu.VMEM((D, 3 * D), BF16),
        pltpu.VMEM((D, D), BF16),
        pltpu.VMEM((S, D), BF16),
        pltpu.VMEM((S, D), BF16),
        pltpu.VMEM((NRB, D, RB), BF16),
        pltpu.VMEM((S, D), BF16),
        pltpu.VMEM((G, S, W), F32),
        pltpu.VMEM((G, 1, W), F32),
        pltpu.VMEM((G, NC, 8, W), F32),
        pltpu.VMEM((G, 128, 128), F32),
        pltpu.VMEM((8, D), F32),
        pltpu.VMEM((G, 256, 128), BF16),
        pltpu.VMEM((S, 2 * D), BF16),
        pltpu.SMEM((1,), jnp.int32),
        pltpu.SemaphoreType.DMA((6,)),
        pltpu.SemaphoreType.DMA((NRB,)),
    ]
    return pl.pallas_call(
        _kernel,
        out_shape=jax.ShapeDtypeStruct((1, S, 2 * D), BF16),
        in_specs=[any_spec] * 6,
        out_specs=any_spec,
        scratch_shapes=scratch,
        compiler_params=pltpu.CompilerParams(vmem_limit_bytes=110 * 1024 * 1024),
    )(A_x, A_wqkv, A_wo, B_x, B_wqkv, B_wo)
```

```python
import math

import jax
import jax.numpy as jnp
from jax import lax
import jax.experimental.pallas as pl
import jax.experimental.pallas.tpu as pltpu

S = 2048
D = 1024
DH = 32
G = 8
TQ = 128
NQ = S // TQ
CK = 128
NC = S // CK
W = 4 * TQ
RB = 512
NRB = S // RB
CPB = RB // CK
WC = 512
NSPLIT = 2
SP = RB // NSPLIT
UR = 256
KRAW = 768

F32 = jnp.float32
BF16 = jnp.bfloat16
NT = (((1,), (1,)), ((), ()))
TN = (((0,), (0,)), ((), ()))
QSCALE = (DH ** -0.5) * math.log2(math.e)


def _dot(a, b):
    return jnp.dot(a, b, preferred_element_type=F32)


def _phi(t):
    t = t.astype(BF16).astype(F32)
    return jnp.where(t > 0, t + 1.0, jnp.exp(t)) + 1e-6


def _rows(i, n):
    if isinstance(i, int):
        return pl.ds(i * n, n)
    return pl.ds(pl.multiple_of(i * n, n), n)


def _kernel(xa_hbm, wa_hbm, woa_hbm, xb_hbm, wb_hbm, wob_hbm, out_hbm,
            xq, wa, woa, xb, wb, wob,
            q_s, k_s, vt_s, ot_s, sbufs, m_s,
            vb_s, zb_s, w2_s, zer_s, zero_ref,
            xa_sems, wa_sems, in_sems, out_sems, *l_s):
    xa = xq.at[0]
    qb_s = xq.at[1]
    kb_s = q_s
    oa_st = xa
    ob_st = k_s
    on_s = vb_s

    def xa_copy(i, r0, n):
        rows = pl.ds(r0, n)
        return pltpu.make_async_copy(xa_hbm.at[0, rows, :], xa.at[rows, :], xa_sems.at[i])

    def wa_copy(i, c0, n):
        cols = pl.ds(c0, n)
        return pltpu.make_async_copy(wa_hbm.at[:, cols], wa.at[:, cols], wa_sems.at[i])

    def blk(i):
        return pl.ds(i * 512, 512)

    pairs = [(wb_hbm.at[:, blk(i)], wb.at[:, blk(i)]) for i in (4, 5, 0, 1)]
    pairs += [(xb_hbm.at[0, blk(i), :], xb.at[blk(i), :]) for i in range(4)]
    pairs += [(wb_hbm.at[:, blk(i)], wb.at[:, blk(i)]) for i in (2, 3)]
    pairs += [(woa_hbm.at[blk(i), :], woa.at[blk(i), :]) for i in range(2)]
    pairs += [(wob_hbm.at[blk(i), :], wob.at[blk(i), :]) for i in range(2)]
    others = [pltpu.make_async_copy(s, d, in_sems.at[i]) for i, (s, d) in enumerate(pairs)]
    mid = others[:8]
    late = others[8:]

    def qkv_piece(rb, r0, n, c0, nc):
        rows = pl.ds(rb * RB + r0, n) if isinstance(rb, int) else _rows(rb, RB)
        r = _dot(xa[rows, :], wa[:, c0:c0 + nc])
        if c0 < D:
            q_s[rows, c0:c0 + nc] = (r * QSCALE).astype(BF16)
        elif c0 < 2 * D:
            k_s[rows, c0 - D:c0 - D + nc] = r.astype(BF16)
        else:
            vt_s[rb, c0 - 2 * D:c0 - 2 * D + nc, r0:r0 + n] = r.T.astype(BF16)

    x0a, x0b = xa_copy(0, 0, 256), xa_copy(1, 256, 256)
    xr = [xa_copy(rb + 1, rb * RB, RB) for rb in range(1, NRB)]
    wq0, wq1, wq2 = wa_copy(0, 0, 256), wa_copy(1, 256, 256), wa_copy(2, 512, 512)
    wv0, wk0 = wa_copy(3, 2048, 512), wa_copy(4, 1024, 512)
    wv1, wk1 = wa_copy(5, 2560, 512), wa_copy(6, 1536, 512)

    for cp in (x0a, wq0, wq1, x0b):
        cp.start()
    zero_ref[0] = 0
    zer_s[...] = jnp.zeros(zer_s.shape, F32)
    x0a.wait()
    wq0.wait()
    wq2.start()
    qkv_piece(0, 0, 256, 0, 256)
    wq1.wait()
    wv0.start()
    qkv_piece(0, 0, 256, 256, 256)
    x0b.wait()
    wk0.start()
    qkv_piece(0, 256, 256, 0, 512)
    wq2.wait()
    qkv_piece(0, 0, RB, 512, 512)
    wv0.wait()
    wk0.wait()
    for cp in (wv1, wk1, xr[0]):
        cp.start()
    qkv_piece(0, 0, RB, 2048, 512)
    qkv_piece(0, 0, RB, 1024, 512)
    wv1.wait()
    wk1.wait()
    for cp in (xr[1], xr[2], mid[0], mid[1]):
        cp.start()
    qkv_piece(0, 0, RB, 2560, 512)
    qkv_piece(0, 0, RB, 1536, 512)
    for cp in xr:
        cp.wait()

    def qkv_a(rb, carry):
        for i, cp in enumerate(mid[2:]):
            @pl.when(rb == i // 3 + 1)
            def _(cp=cp):
                cp.start()
        for cb in (4, 5, 0, 1, 2, 3):
            qkv_piece(rb, 0, RB, cb * WC, WC)
        return carry

    lax.fori_loop(1, NRB, qkv_a, 0)

    lane_head = lax.broadcasted_iota(jnp.int32, (TQ, 128), 1) // DH

    def get_qm(j, g):
        qf = q_s[_rows(j, TQ), g * 128:(g + 1) * 128].astype(F32)
        return jnp.concatenate(
            [jnp.where(lane_head == h, qf, 0.0) for h in range(4)], axis=0).astype(BF16)

    def a_chunk(g, qm, c, macc):
        kc = k_s[c * CK:(c + 1) * CK, g * 128:(g + 1) * 128]
        s = lax.dot_general(kc, qm, NT, preferred_element_type=F32)
        sbufs[g, c * CK:(c + 1) * CK, :] = s
        cm = jnp.max(s.reshape(CK // 8, 8, W), axis=0)
        return cm if macc is None else jnp.maximum(macc, cm)

    def a_final(g, macc):
        m_s[g] = jnp.max(macc, axis=0, keepdims=True)

    def b_chunk(g, c, m, accs):
        s = sbufs[g, c * CK:(c + 1) * CK, :]
        p = jnp.exp2(s - m)
        n = CK // 8
        cl = p[8 * (n - 1):8 * n, :]
        for i in range(n - 2, -1, -1):
            cl = cl + p[8 * i:8 * i + 8, :]
        l_s[g][c] = cl
        new = []
        for h in range(4):
            r0 = (g * 4 + h) * DH
            c0 = (c % CPB) * CK
            vt = vt_s[c // CPB, r0:r0 + DH, c0:c0 + CK]
            d = _dot(vt, p[:, h * TQ:(h + 1) * TQ].astype(BF16))
            new.append((zer_s[...] if accs is None else accs[h]) + d)
        return new

    def b_final(j, g, accs, z):
        lacc = jnp.sum(l_s[g][pl.ds(z, NC)], axis=0)
        r = 1.0 / jnp.sum(lacc, axis=0, keepdims=True)
        for h in range(4):
            r0 = (g * 4 + h) * DH
            ot_s[j, r0:r0 + DH, :] = (accs[h] * r[:, h * TQ:(h + 1) * TQ]).astype(BF16)

    def make_filler(jobs):
        todo = [(kind, t, n, half) for kind, t in jobs for n in range(G) for half in (0, 1)]
        state = {}

        def step():
            kind, t, n, half = todo.pop(0)
            c0 = {"q": 0, "k": D, "v": 2 * D}[kind] + n * 128
            k0 = half * 512
            rows = _rows(t, 128)
            part = _dot(xb[rows, k0:k0 + 512], wb[k0:k0 + 512, c0:c0 + 128])
            if half == 0:
                state["part0"] = jnp.concatenate([zer_s[...]] * 4, axis=0) + part
            else:
                dst = {"q": qb_s, "k": kb_s, "v": vb_s}[kind]
                dst[rows, n * 128:(n + 1) * 128] = (state["part0"] + part).astype(BF16)

        return step

    for g in range(G):
        qm = get_qm(0, g)
        macc = None
        for c in range(NC):
            macc = a_chunk(g, qm, c, macc)
        a_final(g, macc)
    for cp in mid:
        cp.wait()

    def att_body(j, carry):
        for i, cp in enumerate(late):
            @pl.when(j == i + 1)
            def _(cp=cp):
                cp.start()
        z = zero_ref[0]
        fill = make_filler([("v", j), ("q", j)])
        for g in range(G):
            m = m_s[g]
            qm = get_qm(j + 1, g)
            accs = None
            macc = None
            for c in range(NC):
                if c % 4 == 0:
                    fill()
                accs = b_chunk(g, c, m, accs)
                macc = a_chunk(g, qm, c, macc)
            b_final(j, g, accs, z)
            a_final(g, macc)
        return carry

    lax.fori_loop(0, NQ - 1, att_body, 0)
    for cp in late:
        cp.wait()

    z = zero_ref[0]
    fill = make_filler([("v", NQ - 1), ("q", NQ - 1)] + [("k", t) for t in range(KRAW // 128)])
    for g in range(G):
        m = m_s[g]
        accs = None
        for c in range(NC):
            fill()
            accs = b_chunk(g, c, m, accs)
        b_final(NQ - 1, g, accs, z)

    bd = (lax.broadcasted_iota(jnp.int32, (128, 128), 0) // DH
          == lax.broadcasted_iota(jnp.int32, (128, 128), 1) // DH)

    def finish(g, kg):
        cols = slice(g * 128, (g + 1) * 128)
        pk = jnp.concatenate(
            [_phi(kb_s[0:KRAW, cols]).astype(BF16), _phi(kg).astype(BF16)], axis=0)
        zg = jnp.sum(jnp.sum(pk.astype(F32).reshape(S // 128, 128, 128), axis=0),
                     axis=0, keepdims=True)
        zb_s[cols, :] = jnp.broadcast_to(zg.astype(BF16).astype(F32), (128, 128)).T
        kv = lax.dot_general(pk, vb_s[:, cols], TN, preferred_element_type=F32)
        kv = jnp.where(bd, kv, 0.0).astype(BF16)
        w2_s[cols, :] = _dot(kv, wob[cols, :]).astype(BF16)

    prev = None
    for g in range(G):
        kg = _dot(xb[KRAW:S, :], wb[:, D + g * 128:D + (g + 1) * 128])
        if prev is not None:
            finish(*prev)
        prev = (g, kg)
    finish(*prev)

    def out_copy(i, r0, n, half):
        rows = pl.ds(r0, n)
        src = ob_st if half else oa_st
        return pltpu.make_async_copy(
            src.at[rows, :], out_hbm.at[0, rows, pl.ds(half * D, D)], out_sems.at[i])

    def out_body(rb, carry):
        z = zero_ref[0]
        nt = UR // 128
        units = [(u, g) for u in range(RB // UR) for g in range(G)]

        def urows(u):
            return pl.ds(pl.multiple_of(rb * RB + u * UR, UR), UR)

        def norm(u, g):
            cols = slice(g * 128, (g + 1) * 128)
            pqt = _phi(xq[1 + z, urows(u), cols].T).astype(BF16).astype(F32)
            zb = jnp.concatenate([zb_s[cols, :]] * nt, axis=1)
            den = jnp.sum((pqt * zb).reshape(4, DH, UR), axis=1, keepdims=True)
            ogt = (pqt.reshape(4, DH, UR) * (1.0 / (den + 1e-6))).reshape(128, UR)
            on_s[urows(u), cols] = ogt.astype(BF16).T

        oas = [jnp.concatenate([ot_s[4 * rb + u * nt + i].T for i in range(nt)], axis=0)
               for u in range(RB // UR)]
        norm(*units[0])
        for i, (u, g) in enumerate(units):
            if i + 1 < len(units):
                norm(*units[i + 1])
            cols = slice(g * 128, (g + 1) * 128)
            oa_st[urows(u), cols] = _dot(oas[u], woa[:, cols]).astype(BF16)
        out_copy(rb, pl.multiple_of(rb * RB, RB), RB, 0).start()
        for i in range(NSPLIT):
            rr = pl.multiple_of(rb * RB + i * SP, SP)
            ob_st[pl.ds(rr, SP), :] = _dot(on_s[pl.ds(rr, SP), :], w2_s[...]).astype(BF16)
            out_copy(NRB + rb * NSPLIT + i, rr, SP, 1).start()
        return carry

    lax.fori_loop(0, NRB, out_body, 0)
    for rb in range(NRB):
        out_copy(rb, rb * RB, RB, 0).wait()
    for i in range(NRB * NSPLIT):
        out_copy(NRB + i, i * SP, SP, 1).wait()


@jax.jit
def pallas_concat_heads__mha_block__linear_attn_block__prompt_kernel(
    A_x: jax.Array,
    A_wqkv: jax.Array,
    A_wo: jax.Array,
    B_x: jax.Array,
    B_wqkv: jax.Array,
    B_wo: jax.Array,
):
    any_spec = pl.BlockSpec(memory_space=pl.ANY)
    scratch = [
        pltpu.VMEM((2, S, D), BF16),
        pltpu.VMEM((D, 3 * D), BF16),
        pltpu.VMEM((D, D), BF16),
        pltpu.VMEM((S, D), BF16),
        pltpu.VMEM((D, 3 * D), BF16),
        pltpu.VMEM((D, D), BF16),
        pltpu.VMEM((S, D), BF16),
        pltpu.VMEM((S, D), BF16),
        pltpu.VMEM((NRB, D, RB), BF16),
        pltpu.VMEM((NQ, D, TQ), BF16),
        pltpu.VMEM((G, S, W), F32),
        pltpu.VMEM((G, 1, W), F32),
        pltpu.VMEM((S, D), BF16),
        pltpu.VMEM((D, 128), F32),
        pltpu.VMEM((D, D), BF16),
        pltpu.VMEM((DH, TQ), F32),
        pltpu.SMEM((1,), jnp.int32),
        pltpu.SemaphoreType.DMA((NRB + 1,)),
        pltpu.SemaphoreType.DMA((7,)),
        pltpu.SemaphoreType.DMA((14,)),
        pltpu.SemaphoreType.DMA((NRB + NRB * NSPLIT,)),
    ] + [pltpu.VMEM((NC, 8, W), F32) for _ in range(G)]
    return pl.pallas_call(
        _kernel,
        out_shape=jax.ShapeDtypeStruct((1, S, 2 * D), BF16),
        in_specs=[any_spec] * 6,
        out_specs=any_spec,
        scratch_shapes=scratch,
        compiler_params=pltpu.CompilerParams(vmem_limit_bytes=110 * 1024 * 1024),
    )(A_x, A_wqkv, A_wo, B_x, B_wqkv, B_wo)
```

```python
import math

import jax
import jax.numpy as jnp
from jax import lax
import jax.experimental.pallas as pl
import jax.experimental.pallas.tpu as pltpu

S = 2048
D = 1024
DH = 32
G = 8
TQ = 128
NQ = S // TQ
CK = 128
NC = S // CK
W = 4 * TQ
RB = 512
NRB = S // RB
CPB = RB // CK
WC = 512
NSPLIT = 4
SP = RB // NSPLIT
UR = 256
LG = 4
KRAW = 768

F32 = jnp.float32
BF16 = jnp.bfloat16
NT = (((1,), (1,)), ((), ()))
TN = (((0,), (0,)), ((), ()))
QSCALE = (DH ** -0.5) * math.log2(math.e)


def _dot(a, b):
    return jnp.dot(a, b, preferred_element_type=F32)


def _phi(t):
    t = t.astype(BF16).astype(F32)
    return jnp.where(t > 0, t + 1.0, jnp.exp(t)) + 1e-6


def _rows(i, n):
    if isinstance(i, int):
        return pl.ds(i * n, n)
    return pl.ds(pl.multiple_of(i * n, n), n)


def _kernel(xa_hbm, wa_hbm, woa_hbm, xb_hbm, wb_hbm, wob_hbm, out_hbm,
            xq, wa, woa, xb, wb, wob,
            q_s, k_s, vt_s, ot_s, sbufs, m_s,
            vb_s, zb_s, w2_s, zer_s, zero_ref,
            xa_sems, wa_sems, in_sems, out_sems, *l_s):
    xa = xq.at[0]
    qb_s = xq.at[1]
    kb_s = q_s
    oa_st = xa
    ob_st = k_s
    on_s = vb_s

    def xa_copy(i, r0, n):
        rows = pl.ds(r0, n)
        return pltpu.make_async_copy(xa_hbm.at[0, rows, :], xa.at[rows, :], xa_sems.at[i])

    def wa_copy(i, c0, n):
        cols = pl.ds(c0, n)
        return pltpu.make_async_copy(wa_hbm.at[:, cols], wa.at[:, cols], wa_sems.at[i])

    def blk(i):
        return pl.ds(i * 512, 512)

    pairs = [(wb_hbm.at[:, blk(i)], wb.at[:, blk(i)]) for i in (4, 5, 0, 1)]
    pairs += [(xb_hbm.at[0, blk(i), :], xb.at[blk(i), :]) for i in range(4)]
    pairs += [(wb_hbm.at[:, blk(i)], wb.at[:, blk(i)]) for i in (2, 3)]
    pairs += [(woa_hbm.at[blk(i), :], woa.at[blk(i), :]) for i in range(2)]
    pairs += [(wob_hbm.at[blk(i), :], wob.at[blk(i), :]) for i in range(2)]
    others = [pltpu.make_async_copy(s, d, in_sems.at[i]) for i, (s, d) in enumerate(pairs)]
    mid = others[:8]
    late = others[8:]

    def qkv_piece(rb, r0, n, c0, nc):
        rows = pl.ds(rb * RB + r0, n) if isinstance(rb, int) else _rows(rb, RB)
        r = _dot(xa[rows, :], wa[:, c0:c0 + nc])
        if c0 < D:
            q_s[rows, c0:c0 + nc] = (r * QSCALE).astype(BF16)
        elif c0 < 2 * D:
            k_s[rows, c0 - D:c0 - D + nc] = r.astype(BF16)
        else:
            vt_s[rb, c0 - 2 * D:c0 - 2 * D + nc, r0:r0 + n] = r.T.astype(BF16)

    x0a, x0b = xa_copy(0, 0, 256), xa_copy(1, 256, 256)
    xr = [xa_copy(rb + 1, rb * RB, RB) for rb in range(1, NRB)]
    wq0, wq1, wq2 = wa_copy(0, 0, 256), wa_copy(1, 256, 256), wa_copy(2, 512, 512)
    wv0, wk0 = wa_copy(3, 2048, 512), wa_copy(4, 1024, 512)
    wv1, wk1 = wa_copy(5, 2560, 512), wa_copy(6, 1536, 512)

    for cp in (x0a, wq0, wq1, x0b):
        cp.start()
    zero_ref[0] = 0
    zer_s[...] = jnp.zeros(zer_s.shape, F32)
    x0a.wait()
    wq0.wait()
    wq2.start()
    qkv_piece(0, 0, 256, 0, 256)
    wq1.wait()
    wv0.start()
    qkv_piece(0, 0, 256, 256, 256)
    x0b.wait()
    wk0.start()
    qkv_piece(0, 256, 256, 0, 512)
    wq2.wait()
    qkv_piece(0, 0, RB, 512, 512)
    wv0.wait()
    wk0.wait()
    for cp in (wv1, wk1, xr[0]):
        cp.start()
    qkv_piece(0, 0, RB, 2048, 512)
    qkv_piece(0, 0, RB, 1024, 512)
    wv1.wait()
    wk1.wait()
    for cp in (xr[1], xr[2], mid[0], mid[1]):
        cp.start()
    qkv_piece(0, 0, RB, 2560, 512)
    qkv_piece(0, 0, RB, 1536, 512)
    for cp in xr:
        cp.wait()

    def qkv_a(rb, carry):
        for i, cp in enumerate(mid[2:]):
            @pl.when(rb == i // 3 + 1)
            def _(cp=cp):
                cp.start()
        for cb in (4, 5, 0, 1, 2, 3):
            qkv_piece(rb, 0, RB, cb * WC, WC)
        return carry

    lax.fori_loop(1, NRB, qkv_a, 0)

    lane_head = lax.broadcasted_iota(jnp.int32, (TQ, 128), 1) // DH

    def get_qm(j, g):
        qf = q_s[_rows(j, TQ), g * 128:(g + 1) * 128].astype(F32)
        return jnp.concatenate(
            [jnp.where(lane_head == h, qf, 0.0) for h in range(4)], axis=0).astype(BF16)

    def a_chunk(g, qm, c, macc):
        kc = k_s[c * CK:(c + 1) * CK, g * 128:(g + 1) * 128]
        s = lax.dot_general(kc, qm, NT, preferred_element_type=F32)
        sbufs[g, c * CK:(c + 1) * CK, :] = s
        cm = jnp.max(s.reshape(CK // 8, 8, W), axis=0)
        return cm if macc is None else jnp.maximum(macc, cm)

    def a_final(g, macc):
        m_s[g] = jnp.max(macc, axis=0, keepdims=True)

    def b_chunk(g, c, m, state):
        accs, lrun = state
        s = sbufs[g, c * CK:(c + 1) * CK, :]
        p = jnp.exp2(s - m)
        n = CK // 8
        cl = p[8 * (n - 1):8 * n, :]
        if c % LG:
            cl = cl + lrun
        for i in range(n - 2, -1, -1):
            cl = cl + p[8 * i:8 * i + 8, :]
        if c % LG == LG - 1:
            l_s[g][c // LG] = cl
        new = []
        for h in range(4):
            r0 = (g * 4 + h) * DH
            c0 = (c % CPB) * CK
            vt = vt_s[c // CPB, r0:r0 + DH, c0:c0 + CK]
            d = _dot(vt, p[:, h * TQ:(h + 1) * TQ].astype(BF16))
            new.append((zer_s[...] if accs is None else accs[h]) + d)
        return new, cl

    def b_final(j, g, accs, z):
        lacc = jnp.sum(l_s[g][pl.ds(z, NC // LG)], axis=0)
        r = 1.0 / jnp.sum(lacc, axis=0, keepdims=True)
        for h in range(4):
            r0 = (g * 4 + h) * DH
            ot_s[j, r0:r0 + DH, :] = (accs[h] * r[:, h * TQ:(h + 1) * TQ]).astype(BF16)

    def make_filler(jobs):
        todo = [(kind, t, n, half) for kind, t in jobs for n in range(G) for half in (0, 1)]
        state = {}

        def step():
            kind, t, n, half = todo.pop(0)
            c0 = {"q": 0, "k": D, "v": 2 * D}[kind] + n * 128
            k0 = half * 512
            rows = _rows(t, 128)
            part = _dot(xb[rows, k0:k0 + 512], wb[k0:k0 + 512, c0:c0 + 128])
            if half == 0:
                state["part0"] = jnp.concatenate([zer_s[...]] * 4, axis=0) + part
            else:
                dst = {"q": qb_s, "k": kb_s, "v": vb_s}[kind]
                dst[rows, n * 128:(n + 1) * 128] = (state["part0"] + part).astype(BF16)

        return step

    for g in range(G):
        qm = get_qm(0, g)
        macc = None
        for c in range(NC):
            macc = a_chunk(g, qm, c, macc)
        a_final(g, macc)
    for cp in mid:
        cp.wait()

    def att_body(j, carry):
        for i, cp in enumerate(late):
            @pl.when(j == i + 1)
            def _(cp=cp):
                cp.start()
        z = zero_ref[0]
        fill = make_filler([("v", j), ("q", j)])
        for g in range(G):
            m = m_s[g]
            qm = get_qm(j + 1, g)
            state = (None, None)
            macc = None
            for c in range(NC):
                if c % 4 == 0:
                    fill()
                state = b_chunk(g, c, m, state)
                macc = a_chunk(g, qm, c, macc)
            b_final(j, g, state[0], z)
            a_final(g, macc)
        return carry

    lax.fori_loop(0, NQ - 1, att_body, 0)
    for cp in late:
        cp.wait()

    z = zero_ref[0]
    fill = make_filler([("v", NQ - 1), ("q", NQ - 1)] + [("k", t) for t in range(KRAW // 128)])
    for g in range(G):
        m = m_s[g]
        state = (None, None)
        for c in range(NC):
            fill()
            state = b_chunk(g, c, m, state)
        b_final(NQ - 1, g, state[0], z)

    bd = (lax.broadcasted_iota(jnp.int32, (128, 128), 0) // DH
          == lax.broadcasted_iota(jnp.int32, (128, 128), 1) // DH)

    def finish(g, kg):
        cols = slice(g * 128, (g + 1) * 128)
        pk = jnp.concatenate(
            [_phi(kb_s[0:KRAW, cols]).astype(BF16), _phi(kg).astype(BF16)], axis=0)
        zg = jnp.sum(jnp.sum(pk.astype(F32).reshape(S // 128, 128, 128), axis=0),
                     axis=0, keepdims=True)
        zb_s[cols, :] = jnp.broadcast_to(zg.astype(BF16).astype(F32), (128, 128)).T
        kv = lax.dot_general(pk, vb_s[:, cols], TN, preferred_element_type=F32)
        kv = jnp.where(bd, kv, 0.0).astype(BF16)
        w2_s[cols, :] = _dot(kv, wob[cols, :]).astype(BF16)

    prev = None
    for g in range(G):
        kg = _dot(xb[KRAW:S, :], wb[:, D + g * 128:D + (g + 1) * 128])
        if prev is not None:
            finish(*prev)
        prev = (g, kg)
    finish(*prev)

    def out_copy(i, r0, n, half):
        rows = pl.ds(r0, n)
        src = ob_st if half else oa_st
        return pltpu.make_async_copy(
            src.at[rows, :], out_hbm.at[0, rows, pl.ds(half * D, D)], out_sems.at[i])

    def out_body(rb, carry):
        z = zero_ref[0]
        nt = UR // 128
        units = [(u, g) for u in range(RB // UR) for g in range(G)]

        def urows(u):
            return pl.ds(pl.multiple_of(rb * RB + u * UR, UR), UR)

        def norm(u, g):
            cols = slice(g * 128, (g + 1) * 128)
            pqt = _phi(xq[1 + z, urows(u), cols].T).astype(BF16).astype(F32)
            zb = jnp.concatenate([zb_s[cols, :]] * nt, axis=1)
            den = jnp.sum((pqt * zb).reshape(4, DH, UR), axis=1, keepdims=True)
            ogt = (pqt.reshape(4, DH, UR) * (1.0 / (den + 1e-6))).reshape(128, UR)
            on_s[urows(u), cols] = ogt.astype(BF16).T

        oas = [jnp.concatenate([ot_s[4 * rb + u * nt + i].T for i in range(nt)], axis=0)
               for u in range(RB // UR)]
        norm(*units[0])
        for i, (u, g) in enumerate(units):
            if i + 1 < len(units):
                norm(*units[i + 1])
            cols = slice(g * 128, (g + 1) * 128)
            oa_st[urows(u), cols] = _dot(oas[u], woa[:, cols]).astype(BF16)
        out_copy(rb, pl.multiple_of(rb * RB, RB), RB, 0).start()
        for i in range(NSPLIT):
            rr = pl.multiple_of(rb * RB + i * SP, SP)
            ob_st[pl.ds(rr, SP), :] = _dot(on_s[pl.ds(rr, SP), :], w2_s[...]).astype(BF16)
            out_copy(NRB + rb * NSPLIT + i, rr, SP, 1).start()
        return carry

    lax.fori_loop(0, NRB, out_body, 0)
    for rb in range(NRB):
        out_copy(rb, rb * RB, RB, 0).wait()
    for i in range(NRB * NSPLIT):
        out_copy(NRB + i, i * SP, SP, 1).wait()


@jax.jit
def pallas_concat_heads__mha_block__linear_attn_block__prompt_kernel(
    A_x: jax.Array,
    A_wqkv: jax.Array,
    A_wo: jax.Array,
    B_x: jax.Array,
    B_wqkv: jax.Array,
    B_wo: jax.Array,
):
    any_spec = pl.BlockSpec(memory_space=pl.ANY)
    scratch = [
        pltpu.VMEM((2, S, D), BF16),
        pltpu.VMEM((D, 3 * D), BF16),
        pltpu.VMEM((D, D), BF16),
        pltpu.VMEM((S, D), BF16),
        pltpu.VMEM((D, 3 * D), BF16),
        pltpu.VMEM((D, D), BF16),
        pltpu.VMEM((S, D), BF16),
        pltpu.VMEM((S, D), BF16),
        pltpu.VMEM((NRB, D, RB), BF16),
        pltpu.VMEM((NQ, D, TQ), BF16),
        pltpu.VMEM((G, S, W), F32),
        pltpu.VMEM((G, 1, W), F32),
        pltpu.VMEM((S, D), BF16),
        pltpu.VMEM((D, 128), F32),
        pltpu.VMEM((D, D), BF16),
        pltpu.VMEM((DH, TQ), F32),
        pltpu.SMEM((1,), jnp.int32),
        pltpu.SemaphoreType.DMA((NRB + 1,)),
        pltpu.SemaphoreType.DMA((7,)),
        pltpu.SemaphoreType.DMA((14,)),
        pltpu.SemaphoreType.DMA((NRB + NRB * NSPLIT,)),
    ] + [pltpu.VMEM((NC // LG, 8, W), F32) for _ in range(G)]
    return pl.pallas_call(
        _kernel,
        out_shape=jax.ShapeDtypeStruct((1, S, 2 * D), BF16),
        in_specs=[any_spec] * 6,
        out_specs=any_spec,
        scratch_shapes=scratch,
        compiler_params=pltpu.CompilerParams(vmem_limit_bytes=110 * 1024 * 1024),
    )(A_x, A_wqkv, A_wo, B_x, B_wqkv, B_wo)
```
